```python
import os as _os
_os.environ.setdefault('JAX_PLATFORMS', 'cpu')
import jax
import jax.numpy as jnp

def _softmax(x, axis=-1):
    return jax.nn.softmax(x, axis=axis)

def _gelu(x):
    return jax.nn.gelu(x, approximate=True)

def _silu(x):
    return jax.nn.silu(x)

def _sigmoid(x):
    return jax.nn.sigmoid(x)

def _layernorm(x, axis=-1, eps=1e-05):
    m = jnp.mean(x, axis=axis, keepdims=True)
    v = jnp.var(x, axis=axis, keepdims=True)
    return (x - m) / jnp.sqrt(v + eps)

def _scatter_add(tgt, idx, src, axis=0):
    return tgt.at[idx].add(src)

def _segment_sum(src, seg, n):
    return jax.ops.segment_sum(src, seg, n)

class _Rng:

    def __init__(self, key):
        self._k = key

    def _next(self):
        self._k, sub = jax.random.split(self._k)
        return sub

    def normal(self, shape):
        return jax.random.normal(self._next(), shape, dtype=jnp.bfloat16)

    def randint(self, lo, hi, shape):
        return jax.random.randint(self._next(), shape, lo, hi, dtype=jnp.int32)

    def uniform(self, shape, lo=0.0, hi=1.0):
        return jax.random.uniform(self._next(), shape, jnp.bfloat16, lo, hi)

    def permutation(self, n):
        return jax.random.permutation(self._next(), n)
kernel_name = 'adaLN_cond__sliding_local_dilated__dense_activation_relu__prompt'

def setup_inputs():
    _rng = _Rng(jax.random.key(int.from_bytes(__import__("os").urandom(4), "little")))
    _w = lambda a: (lambda t: t.astype(jnp.bfloat16) if jnp.issubdtype(t.dtype, jnp.floating) else t)(jnp.asarray(a))

    def _A_setup():
        B, S, D = (1, 2048, 576)
        return {'x': _w((lambda *s: _rng.normal(s) * 0.05)(B, S, D)), 'wqkv': _w((lambda *s: _rng.normal(s) * 0.05)(D, 3 * D)), 'wo': _w((lambda *s: _rng.normal(s) * 0.05)(D, D))}
    _A_in = _A_setup()

    def _B_setup():
        B, S, D, Dff = (1, 2048, 576, 4608)
        return {'x': _w((lambda *s: _rng.normal(s) * 0.05)(B, S, D)), 'w1': _w((lambda *s: _rng.normal(s) * 0.05)(D, Dff)), 'w2': _w((lambda *s: _rng.normal(s) * 0.05)(Dff, D))}
    _B_in = _B_setup()
    return {'A_x': _A_in['x'], 'A_wqkv': _A_in['wqkv'], 'A_wo': _A_in['wo'], 'B_x': _B_in['x'], 'B_w1': _B_in['w1'], 'B_w2': _B_in['w2'], 'c': _w((lambda *s: _rng.normal(s) * 0.05)(1, 576) * 8.0), 'w_mod': _w((lambda *s: _rng.normal(s) * 0.05)(576, 6 * 576) * 576 ** (-0.5) * 8.0)}

def reference(A_x, A_wqkv, A_wo, B_x, B_w1, B_w2, c, w_mod):

    def _A_ref(x, wqkv, wo):
        B, S, D = x.shape
        H = 32
        Dh = D // H
        W, dil = (8, 2)
        qkv = (lambda x, *d: x.transpose(*d))((x @ wqkv).reshape(B, S, 3, H, Dh), 2, 0, 3, 1, 4)
        q, k, v = (qkv[0], qkv[1], qkv[2])
        scale = Dh ** (-0.5)
        pos = jnp.arange(S)
        off = jnp.arange(W) * dil
        idx = pos[:, None] - off[None, :]
        mask = idx >= 0
        idx_c = jnp.where(mask, idx, 0).reshape(-1)
        kg = k[:, :, idx_c, :].reshape(B, H, S, W, Dh)
        vg = v[:, :, idx_c, :].reshape(B, H, S, W, Dh)
        logits = jnp.einsum('bhsd,bhswd->bhsw', q, kg) * scale
        logits = jnp.where(mask[None, None, :, :], logits, -1000000000.0)
        attn = _softmax(logits, axis=-1)
        o = jnp.einsum('bhsw,bhswd->bhsd', attn, vg)
        return (lambda x, *d: x.transpose(*d))(o, 0, 2, 1, 3).reshape(B, S, D) @ wo

    def _B_ref(x, w1, w2):
        h = jnp.einsum('bsd,df->bsf', x, w1)
        zero = jnp.zeros_like(h)
        h = jnp.maximum(h, zero)
        return jnp.einsum('bsf,fd->bsd', h, w2)
    x = A_x
    mod = (_silu(c) @ w_mod).reshape(c.shape[0], 6, 1, -1)
    sa, ca, ga, sb, cb, gb = (mod[:, 0].copy(), mod[:, 1].copy(), mod[:, 2].copy(), mod[:, 3].copy(), mod[:, 4].copy(), mod[:, 5].copy())
    h = _layernorm(x, axis=-1) * (1 + ca) + sa
    x = x + ga * _A_ref(h, A_wqkv, A_wo)
    h = _layernorm(x, axis=-1) * (1 + cb) + sb
    x = x + gb * _B_ref(h, B_w1, B_w2)
    return x
```

```python
import functools
import math
import numpy as np

import jax
import jax.numpy as jnp
import jax.experimental.pallas as pl
import jax.experimental.pallas.tpu as pltpu

f32 = jnp.float32
bf16 = jnp.bfloat16

S, D, H, DH, W, DIL, F = 2048, 576, 32, 18, 8, 2, 4608
EPS = 1e-5
SCALE = DH ** -0.5
NT = (((1,), (1,)), ((), ()))

SB = 512
NB = S // SB
HALO = 16
RB = 16
FC = 512
LO = True
FINE = True
SER = True
HI = False
NQ = 1792


def _tie32(a, z):
    if z is None:
        return a
    n = a.shape[0] // 8
    a3 = pltpu.bitcast(a, jnp.uint32).reshape(n, 8, 128) | z[None]
    return pltpu.bitcast(a3.reshape(n * 8, 128), f32)


CH = 64


def _bc8(row):
    return jnp.broadcast_to(row, (8, 128))


def _rep(a8, n):
    return jnp.concatenate([a8] * (n // 8), axis=0)


def _fold8(a):
    parts = [a[r:r + 8] for r in range(0, a.shape[0], 8)]
    while len(parts) > 1:
        parts = [parts[i] + parts[i + 1] for i in range(0, len(parts), 2)]
    return parts[0]


def _ln_stats(load, z=None):
    x0 = s1 = s2 = None
    for a in range(0, D, CH):
        x = load(a)
        if x0 is None:
            x0 = _tie32(_bc8(x[0:1, :]), z)
        d = x - _rep(x0, CH)
        s1 = d if s1 is None else s1 + d
        s2 = d * d if s2 is None else s2 + d * d
    m = jnp.sum(_fold8(s1), axis=0, keepdims=True) * (1.0 / D)
    e2 = jnp.sum(_fold8(s2), axis=0, keepdims=True) * (1.0 / D)
    var = jnp.maximum(e2 - m * m, 0.0)
    return x0 + _bc8(m), _bc8(jax.lax.rsqrt(var + EPS))


def _ln_apply(load, mean, rstd, scale_ref, shift_ref, dst_ref, row0):
    for c0 in range(0, D, 128):
        cw = min(128, D - c0)
        outs = []
        for a in range(c0, c0 + cw, CH):
            xn = (load(a) - _rep(mean, CH)) * _rep(rstd, CH)
            outs.append(xn * scale_ref[a:a + CH, :] + shift_ref[a:a + CH, :])
        blk = outs[0] if len(outs) == 1 else jnp.concatenate(outs, axis=0)
        dst_ref[c0 // 128, row0:row0 + 128, 0:cw] = blk.T.astype(bf16)


def _cat5(ref, r0, r1):
    return jnp.concatenate([ref[kt, r0:r1, :] for kt in range(4)] + [ref[4, r0:r1, 0:64]], axis=1)


def _kernel(c_hbm, x_hbm, wqkv_hbm, wo_hbm, w1_hbm, w2t_hbm, wmod_hbm, out_hbm,
            x_v, wqkv_v, wo_v, w1_v, w2t_v, wmod_v, out_v,
            wq32, wqp, wop, mod_v, h_v, kva, o_v, x1_v, hn_v, sct_v, c_v, sems, osems):
    def cp(src, dst, i):
        return pltpu.make_async_copy(src, dst, sems.at[i])

    def cols(src, dst, c0, n, i):
        return cp(src.at[:, pl.ds(c0, n)], dst.at[pl.ds(0, D), pl.ds(c0, n)], i)

    c_wq = cols(wqkv_hbm, wqkv_v, 0, 640, 0)
    c_wkv = cols(wqkv_hbm, wqkv_v, 640, 1088, 6 + NB)
    c_wm0 = cols(wmod_hbm, wmod_v, 0, 1152, 1)
    c_x = [cp(x_hbm.at[:, pl.ds(i * SB, SB)], x_v.at[i], 2 + i) for i in range(NB)]
    c_wo = cp(wo_hbm, wo_v.at[pl.ds(0, D), :], 2 + NB)
    c_wm1 = cols(wmod_hbm, wmod_v, 1152, 2304, 3 + NB)
    c_w1 = cp(w1_hbm, w1_v, 4 + NB)
    c_w2 = cp(w2t_hbm, w2t_v, 5 + NB)
    c_c = cp(c_hbm, c_v, 8 + NB)
    for cc in (c_c, c_x[0], c_wm0, c_wq, c_wkv, c_x[1], c_x[2], c_wo, c_x[3], c_wm1, c_w1, c_w2):
        cc.start()

    lane8 = jax.lax.broadcasted_iota(jnp.int32, (RB, 128), 1)

    kva[0, 4:14, 0:HALO, :] = jnp.zeros((10, HALO, 128), f32)

    c_c.wait()
    cf = c_v[...].astype(f32)
    sc = cf * jax.nn.sigmoid(cf)
    c8 = _bc8(cf[:, 0:128])
    zmask = jnp.where((c8 > 1.0) & (c8 < -1.0), jnp.uint32(0xFFFFFFFF), jnp.uint32(0))
    for t in range(5):
        kw = 128 if t < 4 else 64
        row = sc[:, t * 128:t * 128 + kw]
        if kw < 128:
            row = jnp.concatenate([row, jnp.zeros((1, 64), f32)], axis=1)
        sct_v[t * 128:t * 128 + kw, :] = jnp.broadcast_to(row, (128, 128)).T[0:kw, :]

    def mod_tile(j, z=None):
        acc = None
        for a in range(0, D, 64):
            p = wmod_v[a:a + 64, j * 128:(j + 1) * 128].astype(f32) * sct_v[a:a + 64, :]
            acc = _tie32(p, z) if acc is None else acc + p
        r = jnp.sum(acc, axis=0, keepdims=True)
        st["mz"] = zof(_bc8(r))
        rt = jnp.broadcast_to(r, (128, 128)).T
        g0 = j * 128
        for a in range(g0, g0 + 128, 64):
            jj = a // D
            val = rt[a - g0:a - g0 + 64, :]
            if jj in (1, 4):
                val = val + 1.0
            mod_v[jj, a - jj * D:a - jj * D + 64, :] = val

    stats0 = []

    def xload(i, t, zb=None):
        def load(a):
            w = x_v[i, a:a + CH, t * 128:(t + 1) * 128]
            if zb is not None:
                w = pltpu.bitcast(pltpu.bitcast(w, jnp.uint32) | _rep(zb, CH // 2), bf16)
            return w.astype(f32)
        return load

    def ln1_stats(i):
        for t in range(SB // 128):
            stats0.append(_ln_stats(xload(i, t)))

    def ln1_apply(i):
        zb = zmask
        for t in range(SB // 128):
            _ln_apply(xload(i, t, zb), *stats0[t], mod_v.at[1], mod_v.at[0], h_v.at[i], t * 128)

    def ln1(i, z=None):
        zb = zmask
        for t in range(SB // 128):
            mean, rstd = _ln_stats(xload(i, t), z)
            _ln_apply(xload(i, t, zb), mean, rstd, mod_v.at[1], mod_v.at[0], h_v.at[i], t * 128)
            if SER:
                z = zof(rstd)

    def tie_tile(a, z):
        if z is None:
            return a
        n = a.shape[0] // 16
        zz = jnp.concatenate([z[:, 0:a.shape[1]]] * n, axis=0)
        return pltpu.bitcast(pltpu.bitcast(a, jnp.uint32) | zz, bf16)

    def prep_t(j0, j1, z=None):
        for j in range(j0, j1):
            nw = 128 if j < 13 else 64
            for kt in range(5):
                kw = 128 if kt < 4 else 64
                t = tie_tile(wqkv_v[kt * 128:kt * 128 + kw, j * 128:j * 128 + nw], z).astype(f32).T
                wq32[kt, j * 128:j * 128 + nw, 0:kw] = t

    def prep_p(p, d0=0, d1=DH):
        for d in range(d0, d1):
            if d < 16:
                row0 = p * 512 + d * 32
            elif p == 0:
                row0 = 1536 + (d - 16) * 32
            elif p == 2:
                row0 = 1536 + 64 + (d - 16) * 32
            else:
                row0 = 1664 + (d - 16) * 32
            for kt in range(5):
                kw = 128 if kt < 4 else 64
                blk = wq32[kt, pl.ds(p * D + d, 32, stride=DH), :]
                wqp[kt, row0:row0 + 32, 0:kw] = blk[:, 0:kw].astype(bf16)
        if p == 1 and d1 == DH:
            wqp[:, 1728:1792, :] = jnp.zeros((5, 64, 128), bf16)

    def prep_wo(z=None):
        for nt in range(5):
            nw = 128 if nt < 4 else 64
            wq32[nt, 0:D, 0:nw] = tie_tile(wo_v[0:D, nt * 128:nt * 128 + nw], z).astype(f32)
        for nt in range(5):
            nw = 128 if nt < 4 else 64
            for tau in range(5):
                if tau < 4:
                    parts = [wq32[nt, pl.ds(4 * tau + g, 32, stride=DH), :] for g in range(4)]
                else:
                    parts = [jnp.zeros((64, 128), f32)] + [
                        wq32[nt, pl.ds(16 + g, 32, stride=DH), :] for g in range(2)]
                blk = jnp.concatenate(parts, axis=0)
                wop[tau, nt * 128:nt * 128 + nw, :] = blk.T[0:nw, :].astype(bf16)

    def qkv_part(i, part, side=None, rows=(0, SB), z=None):
        h = _cat5(h_v.at[i], rows[0], rows[1])
        kv = kva.at[i]
        r0 = HALO + rows[0]
        n = rows[1] - rows[0]
        n0, n1, base = ((0, 512, 0), (512, 1024, 5), (1024, 1536, 10), (1536, 1792, None))[part]
        y = jax.lax.dot_general(h, _cat5(wqp, n0, n1), NT, preferred_element_type=f32)
        if base is not None:
            for t in range(4):
                kv[base + t, r0:r0 + n, :] = y[:, t * 128:(t + 1) * 128]
        else:
            kv[4, r0:r0 + n, :] = y[:, 0:128]
            kv[9, r0:r0 + n, :] = y[:, 128:256]
        if side is not None:
            side(y)
        return y

    def qkv(i, side=None):
        for part in range(4):
            qkv_part(i, part, side)

    def zof(val):
        zm = zmask
        return pltpu.bitcast(val[0:8, 0:128], jnp.uint32) & zm

    def tie16(x, z):
        if z is None:
            return x
        t = pltpu.bitcast(pltpu.bitcast(x[0:16, 0:128], jnp.uint32) | z, bf16)
        row0 = jnp.concatenate([t, x[0:16, 128:]], axis=1)
        return jnp.concatenate([row0, x[16:]], axis=0)

    def zor(a, b):
        return b if a is None else (a if b is None else a | b)

    st = {"lo": None, "hi": None}

    def halo(i):
        kva[i, 4:14, 0:HALO, :] = kva[i - 1, 4:14, SB:SB + HALO, :]

    def gate16(ref, val):
        pass

    LOG2E = 1.4426950408889634
    NG = SB // RB

    def att_a(i, g):
        lr = g * RB
        r = HALO + lr
        kv = kva.at[i]
        acc = [None] * W
        for t in range(5):
            q = kv[t, r:r + RB, :]
            if LO and st["lo"] is not None:
                zl = jnp.concatenate([st["lo"]] * (RB // 8), axis=0)
                q = pltpu.bitcast(pltpu.bitcast(q, jnp.uint32) | zl, f32)
            for w in range(W):
                p = q * kv[5 + t, r - 2 * w:r - 2 * w + RB, :]
                acc[w] = p if acc[w] is None else acc[w] + p
        res = [a + pltpu.roll(a, 64, axis=1) for a in acc]
        st["hi"] = zof(res[W - 1])
        return res

    def att_b(i, g, acc):
        out = []
        s0 = g * RB if (isinstance(i, int) and i == 0) else S
        for w in range(W):
            a = acc[w] + pltpu.roll(acc[w], 32, axis=1)
            if s0 < 2 * w:
                row = jax.lax.broadcasted_iota(jnp.int32, (RB, 128), 0)
                a = jnp.where(row >= 2 * w - s0, a, -1e9 / SCALE)
            out.append(a)
        st["hi"] = zof(out[W - 1])
        return out

    def att_c(i, g, acc):
        lr = g * RB
        r = HALO + lr
        kv = kva.at[i]
        m = acc[0]
        for w in range(1, W):
            m = jnp.maximum(m, acc[w])
        e = [jnp.exp2((a - m) * (SCALE * LOG2E)) for a in acc]
        ssum = e[0]
        for w in range(1, W):
            ssum = ssum + e[w]
        inv = pl.reciprocal(ssum, approx=True)
        inv = inv * (2.0 - ssum * inv)
        for t in range(5):
            o = None
            for w in range(W):
                p = e[w] * kv[(10 + t) if t < 4 else 4, r - 2 * w:r - 2 * w + RB, :]
                o = p if o is None else o + p
            o = o * inv
            if t == 4:
                o = jnp.where(lane8 >= 64, o, 0.0)
            o_v[i, t, lr:lr + RB, :] = o.astype(bf16)
        st["hi"] = zof(o)

    def attn_gen(i):
        sa, sb = {}, {}
        if not (isinstance(i, int) and i == 0):
            halo(i)
        for step in range(NG + 2):
            if step < NG:
                sa[step] = att_a(i, step)
            if 0 <= step - 1 < NG:
                sb[step - 1] = att_b(i, step - 1, sa.pop(step - 1))
            if 0 <= step - 2 < NG:
                att_c(i, step - 2, sb.pop(step - 2))
            yield

    def run(gen, n):
        z = None
        for _ in range(n):
            st["hi"] = None
            next(gen, None)
            z = zor(z, st["hi"])
        st["hi"] = None
        return z

    def wo_ln2(i, work=()):
        yT = jax.lax.dot_general(jnp.concatenate([wop[t] for t in range(5)], axis=1),
                                 jnp.concatenate([o_v[i, t] for t in range(5)], axis=1), NT, preferred_element_type=f32)
        for q, items in enumerate(work):
            z = zof(yT[q * (D // len(work) // 8 * 8):q * (D // len(work) // 8 * 8) + 8])
            for it in items:
                it(z)
        for t in range(SB // 128):
            xl = xload(i, t)

            def load1(a, t=t, xl=xl):
                x1 = xl(a) + mod_v[2, a:a + CH, :] * yT[a:a + CH, t * 128:(t + 1) * 128]
                x1_v[i, t, a:a + CH, :] = x1
                return x1

            def load2(a, t=t):
                return x1_v[i, t, a:a + CH, :]

            mean, rstd = _ln_stats(load1)
            _ln_apply(load2, mean, rstd, mod_v.at[4], mod_v.at[3], hn_v.at[i], t * 128)

    def wcat(ref, f, r0=0, r1=D):
        return ref[r0:r1, f * FC:(f + 1) * FC]

    NTB = SB // 128
    RG = 192

    def out_copy(i, t, r0=0, r1=D, sem=None):
        g = i * NTB + t
        return pltpu.make_async_copy(out_v.at[g, pl.ds(r0, r1 - r0), :],
                                     out_hbm.at[pl.ds(r0, r1 - r0), pl.ds(g * 128, 128)],
                                     osems.at[g] if sem is None else osems.at[sem])

    def epilogue(i, acc, r0, r1):
        for t in range(NTB):
            for a in range(r0, r1, CH):
                x2 = x1_v[i, t, a:a + CH, :] + mod_v[5, a:a + CH, :] * acc[a - r0:a - r0 + CH, t * 128:(t + 1) * 128]
                out_v[i * NTB + t, a:a + CH, :] = x2.astype(bf16)

    def ffn(i, side, last=False):
        hn = _cat5(hn_v.at[i], 0, SB)
        acc = None
        nf = F // FC
        for f in range(nf):
            hp = jnp.dot(hn, wcat(w1_v, f), preferred_element_type=f32)
            hh = jnp.maximum(hp, 0.0).astype(bf16)
            if last and f == nf - 1:
                for k, r0 in enumerate(range(0, D, RG)):
                    p = jax.lax.dot_general(wcat(w2t_v, f, r0, r0 + RG), hh, NT, preferred_element_type=f32)
                    epilogue(i, acc[r0:r0 + RG] + p, r0, r0 + RG)
                    for t in range(NTB):
                        out_copy(i, t, r0, r0 + RG, S // 128 + k * NTB + t).start()
                return
            p = jax.lax.dot_general(wcat(w2t_v, f), hh, NT, preferred_element_type=f32)
            acc = p if acc is None else acc + p
            side(f, nf, hp, p)
        epilogue(i, acc, 0, D)
        for t in range(NTB):
            out_copy(i, t).start()

    c_x[0].wait()
    ln1_stats(0)
    c_wm0.wait()
    for j in range(9):
        mod_tile(j)
    ln1_apply(0)
    c_wq.wait()
    prep_t(0, 5)
    prep_p(0)

    def toks(y, n, k):
        return [zof(y[q * n // k:q * n // k + 8]) for q in range(k)]

    lnst = {}

    def Ls(i, t):
        def f(z):
            lnst[(i, t)] = _ln_stats(xload(i, t), z)
        return f

    def La(i, t):
        def f(z):
            zb = z if z is not None else zmask
            _ln_apply(xload(i, t, zb), *lnst.pop((i, t)), mod_v.at[1], mod_v.at[0], h_v.at[i], t * 128)
        return f

    def ln1_tile(i, t, z):
        zb = zmask
        mean, rstd = _ln_stats(xload(i, t), z)
        _ln_apply(xload(i, t, zb), mean, rstd, mod_v.at[1], mod_v.at[0], h_v.at[i], t * 128)

    gen0 = attn_gen(0)
    NS = NG + 2

    def att(n):
        def f(z):
            st["lo"] = z
            run(gen0, n)
        return f

    def dot(i, part, work, rows=(0, SB)):
        y = qkv_part(i, part, rows=rows)
        zs4 = toks(y, rows[1] - rows[0], max(len(work), 1))
        for q, items in enumerate(work):
            for it in items:
                it(zs4[q])

    L = lambda i, t: (lambda z: ln1_tile(i, t, z))
    M = lambda j: (lambda z: mod_tile(j, z))
    PT = lambda j0, j1: (lambda z: prep_t(j0, j1, z))
    PP = lambda p, d0, d1: (lambda z: prep_p(p, d0, d1))
    A1, A2 = att(1), att(2)

    dot(0, 0, [], rows=(0, 256))
    c_wkv.wait()
    dot(0, 0, [[PT(5, 6)], [PT(6, 7)], [PT(7, 8)], [PT(8, 9)], [PT(9, 10)]], rows=(256, 512))
    prep_p(1)
    dot(0, 1, [[PT(10, 11)], [PT(11, 12)], [PT(12, 13)], [PT(13, 14)], [PP(2, 0, 6)], [PP(2, 6, 12)], [PP(2, 12, 18)], []])
    c_x[1].wait()
    c_x[2].wait()
    dot(0, 2, [[Ls(1, 0)], [La(1, 0)], [Ls(1, 1)], [La(1, 1)], [Ls(1, 2)], [La(1, 2)], [Ls(1, 3)], [La(1, 3)]])
    dot(0, 3, [[Ls(2, 0)], [], [La(2, 0)], []])
    dot(1, 0, [[A1], [Ls(2, 1)], [A1], [La(2, 1)], [A1], [Ls(2, 2)], [A1], [La(2, 2)]])
    dot(1, 1, [[A1], [Ls(2, 3)], [A1], [La(2, 3)], [A1], [], [A1], []])
    c_wo.wait()
    c_x[3].wait()
    c_wm1.wait()
    dot(1, 2, [[A1], [M(9)], [A1], [M(10)], [A1], [M(11)], [A1], [M(12)]])
    dot(1, 3, [[A1], [M(13)], [A1], []])
    dot(2, 0, [[A1], [Ls(3, 0)], [A1], [La(3, 0)], [A1], [Ls(3, 1)], [A1], [La(3, 1)]])
    dot(2, 1, [[A1], [Ls(3, 2)], [A1], [La(3, 2)], [A1], [Ls(3, 3)], [A1], [La(3, 3)]])
    dot(2, 2, [[A1], [], [A1], [prep_wo], [A1], [], [A1], []])
    dot(2, 3, [[A1], [], [A1], []])
    dot(3, 0, [[A1], [M(14)], [A1], [M(15)], [A1], [M(16)], [A1], [M(17)]])
    dot(3, 1, [[A1], [M(18)], [A1], [M(19)], [A1], [M(20)], [], []])
    st["lo"] = None
    run(gen0, NS)
    wo_ln2(0, [[M(21)], [M(22)], [], []])
    dot(3, 2, [[], [], [], [M(23)], [], [M(24)], [], []])
    dot(3, 3, [[M(25)], [M(26)]])
    c_w1.wait()
    c_w2.wait()

    def mk_side(i, last):
        gen = attn_gen(i + 1) if last is False else None

        def side(f, nf, hp, p):
            if gen is None:
                return
            if f < nf - 2:
                toks = [zof(hp[q * SB // 4:q * SB // 4 + 8]) for q in range(4)] if FINE else []
                toks += [zof(p[q * D // 4:q * D // 4 + 8]) for q in range(4 if FINE else 1)]
                per = -(-NS // ((nf - 2) * len(toks)))
                for z in toks:
                    st["lo"] = z
                    run(gen, per)
            if f == nf - 2:
                st["lo"] = None
                run(gen, NS)
                wo_ln2(i + 1)
        return side

    for i in range(NB):
        ffn(i, mk_side(i, i == NB - 1), last=(i == NB - 1))
    for i in range(NB - 1):
        for t in range(NTB):
            out_copy(i, t).wait()
    for k, r0 in enumerate(range(0, D, RG)):
        for t in range(NTB):
            out_copy(NB - 1, t, r0, r0 + RG, S // 128 + k * NTB + t).wait()


@jax.jit
def pallas_adaLN_cond__sliding_local_dilated__dense_activation_relu__prompt_kernel(
    A_x, A_wqkv, A_wo, B_x, B_w1, B_w2, c, w_mod,
):
    del B_x
    xT = A_x.reshape(S, D).T
    w2T = B_w2.T
    anyspec = pl.BlockSpec(memory_space=pl.ANY)
    outT = pl.pallas_call(
        _kernel,
        in_specs=[anyspec] * 7,
        out_specs=anyspec,
        out_shape=jax.ShapeDtypeStruct((D, S), bf16),
        scratch_shapes=[
            pltpu.VMEM((NB, D, SB), bf16),
            pltpu.VMEM((D + 16, 3 * D), bf16),
            pltpu.VMEM((D + 16, D), bf16),
            pltpu.VMEM((D, F), bf16),
            pltpu.VMEM((D, F), bf16),
            pltpu.VMEM((D + 16, 6 * D), bf16),
            pltpu.VMEM((S // 128, D, 128), bf16),
            pltpu.VMEM((5, 1792, 128), f32),
            pltpu.VMEM((5, NQ, 128), bf16),
            pltpu.VMEM((5, D, 128), bf16),
            pltpu.VMEM((6, D, 128), f32),
            pltpu.VMEM((NB, 5, SB, 128), bf16),
            pltpu.VMEM((NB, 14, HALO + SB, 128), f32),
            pltpu.VMEM((NB, 5, SB, 128), bf16),
            pltpu.VMEM((NB, SB // 128, D, 128), f32),
            pltpu.VMEM((NB, 5, SB, 128), bf16),
            pltpu.VMEM((D, 128), f32),
            pltpu.VMEM((1, D), bf16),
            pltpu.SemaphoreType.DMA((9 + NB,)),
            pltpu.SemaphoreType.DMA((S // 128 + 12,)),
        ],
        compiler_params=pltpu.CompilerParams(vmem_limit_bytes=100 * 2 ** 20),
        name="adaln_block",
    )(c, xT, A_wqkv, A_wo, B_w1, w2T, w_mod)
    return outT.T.reshape(1, S, D)
```

```python
import jax
import jax.numpy as jnp
import jax.experimental.pallas as pl
import jax.experimental.pallas.tpu as pltpu

f32 = jnp.float32
bf16 = jnp.bfloat16
u32 = jnp.uint32

S, D, DH, W, F = 2048, 576, 18, 8, 4608
EPS = 1e-5
SCALE = DH ** -0.5
LOG2E = 1.4426950408889634
NT = (((1,), (1,)), ((), ()))

SB = 512
NB = S // SB
NTB = SB // 128
HALO = 16
RB = 16
NG = SB // RB
FC = 512
CH = 64
RS = 256
RGS = ((0, 256), (256, 448), (448, 576))


def _tie(a, z):
    if z is None:
        return a
    n = a.shape[0] // 8
    a3 = pltpu.bitcast(a, u32).reshape(n, 8, 128) | z[None]
    return pltpu.bitcast(a3.reshape(n * 8, 128), f32)


def _tie16(a, z):
    if z is None:
        return a
    zz = jnp.concatenate([z[:, 0:a.shape[1]]] * (a.shape[0] // 16), axis=0)
    return pltpu.bitcast(pltpu.bitcast(a, u32) | zz, bf16)


def _bc8(row):
    return jnp.broadcast_to(row, (8, 128))


def _rep(a8, n):
    return jnp.concatenate([a8] * (n // 8), axis=0)


def _fold8(a):
    parts = [a[r:r + 8] for r in range(0, a.shape[0], 8)]
    while len(parts) > 1:
        parts = [parts[i] + parts[i + 1] for i in range(0, len(parts), 2)]
    return parts[0]


def _ln_stats(load, z=None):
    x0 = s1 = s2 = None
    for a in range(0, D, CH):
        x = load(a)
        if x0 is None:
            x0 = _tie(_bc8(x[0:1, :]), z)
        d = x - _rep(x0, CH)
        s1 = d if s1 is None else s1 + d
        s2 = d * d if s2 is None else s2 + d * d
    m = jnp.sum(_fold8(s1), axis=0, keepdims=True) * (1.0 / D)
    e2 = jnp.sum(_fold8(s2), axis=0, keepdims=True) * (1.0 / D)
    var = jnp.maximum(e2 - m * m, 0.0)
    return x0 + _bc8(m), _bc8(jax.lax.rsqrt(var + EPS))


def _ln_apply(load, mean, rstd, scale_ref, shift_ref, dst_ref, row0, transpose):
    for c0 in range(0, D, 128):
        cw = min(128, D - c0)
        outs = []
        for a in range(c0, c0 + cw, CH):
            xn = (load(a) - _rep(mean, CH)) * _rep(rstd, CH)
            outs.append(xn * scale_ref[a:a + CH, :] + shift_ref[a:a + CH, :])
        blk = outs[0] if len(outs) == 1 else jnp.concatenate(outs, axis=0)
        if transpose:
            dst_ref[c0 // 128, row0:row0 + 128, 0:cw] = blk.T.astype(bf16)
        else:
            dst_ref[row0 // 128, c0:c0 + cw, :] = blk.astype(bf16)


def _cat5(ref, r0, r1):
    return jnp.concatenate([ref[kt, r0:r1, :] for kt in range(4)] + [ref[4, r0:r1, 0:64]], axis=1)


def _kernel(c_hbm, x_hbm, wqkv_hbm, wo_hbm, w1_hbm, w2t_hbm, wmod_hbm, out_hbm,
            x_v, wqkv_v, wo_v, w1_v, w2t_v, wmod_v, out_v,
            wq32, wqp, wop, mod_v, sct_v, c_v, sems, osem, *perblk):
    h_vs, kvs, o_vs, x1_vs, hn_vs = (perblk[k * NB:(k + 1) * NB] for k in range(5))

    def cp(src, dst, i):
        return pltpu.make_async_copy(src, dst, sems.at[i])

    def cols(src, dst, c0, n, i):
        return cp(src.at[:, pl.ds(c0, n)], dst.at[:, pl.ds(c0, n)], i)

    c_c = cp(c_hbm, c_v, 0)
    c_x = [cp(x_hbm.at[:, pl.ds(i * SB, SB)], x_v.at[i], (1, 6, 6, 6)[i]) for i in range(NB)]
    c_wm0 = cols(wmod_hbm, wmod_v, 0, 1152, 2)
    c_wq = cols(wqkv_hbm, wqkv_v, 0, 640, 3)
    c_wk = cols(wqkv_hbm, wqkv_v, 640, 640, 4)
    c_wv = cols(wqkv_hbm, wqkv_v, 1280, 448, 5)
    c_wo = cp(wo_hbm, wo_v, 7)
    c_wm1 = cols(wmod_hbm, wmod_v, 1152, 2304, 7)
    c_w1 = cp(w1_hbm, w1_v, 8)
    c_w2 = cp(w2t_hbm, w2t_v, 8)
    for cc in (c_c, c_wm0, c_x[0], c_wq, c_wk, c_wv, c_x[1], c_x[2], c_x[3], c_wo, c_wm1, c_w1, c_w2):
        cc.start()

    lane = jax.lax.broadcasted_iota(jnp.int32, (RB, 128), 1)
    kvs[0][4:14, 0:HALO, :] = jnp.zeros((10, HALO, 128), f32)

    c_c.wait()
    cf = c_v[...].astype(f32)
    sc = cf * jax.nn.sigmoid(cf)
    c8 = _bc8(cf[:, 0:128])
    zmask = jnp.where((c8 > 1.0) & (c8 < -1.0), jnp.uint32(0xFFFFFFFF), jnp.uint32(0))
    for t in range(5):
        kw = 128 if t < 4 else 64
        row = sc[:, t * 128:t * 128 + kw]
        if kw < 128:
            row = jnp.concatenate([row, jnp.zeros((1, 64), f32)], axis=1)
        sct_v[t * 128:t * 128 + kw, :] = jnp.broadcast_to(row, (128, 128)).T[0:kw, :]

    def zof(val):
        return pltpu.bitcast(val[0:8, 0:128], u32) & zmask

    def mod_tile(j, z=None):
        acc = None
        for a in range(0, D, CH):
            p = wmod_v[a:a + CH, j * 128:(j + 1) * 128].astype(f32) * sct_v[a:a + CH, :]
            acc = _tie(p, z) if acc is None else acc + p
        r = jnp.sum(acc, axis=0, keepdims=True)
        rt = jnp.broadcast_to(r, (128, 128)).T
        g0 = j * 128
        for a in range(g0, g0 + 128, 64):
            jj = a // D
            val = rt[a - g0:a - g0 + 64, :]
            if jj in (1, 4):
                val = val + 1.0
            mod_v[jj, a - jj * D:a - jj * D + 64, :] = val

    def xload(i, t, zb=None):
        def load(a):
            w = x_v[i, a:a + CH, t * 128:(t + 1) * 128]
            if zb is not None:
                w = pltpu.bitcast(pltpu.bitcast(w, u32) | _rep(zb, CH // 2), bf16)
            return w.astype(f32)
        return load

    def prep_w(p, kt, z=None):
        kw = 128 if kt < 4 else 64
        for j in range(*((0, 5), (5, 10), (10, 14))[p]):
            nw = 128 if j < 13 else 64
            t = _tie16(wqkv_v[kt * 128:kt * 128 + kw, j * 128:j * 128 + nw], z).astype(f32).T
            wq32[kt, j * 128:j * 128 + nw, 0:kw] = t
        for d in range(DH):
            if d < 16:
                row0 = p * 512 + d * 32
            elif p == 0:
                row0 = 1536 + (d - 16) * 32
            elif p == 2:
                row0 = 1600 + (d - 16) * 32
            else:
                row0 = 1664 + (d - 16) * 32
            blk = wq32[kt, pl.ds(p * D + d, 32, stride=DH), :]
            wqp[kt, row0:row0 + 32, 0:kw] = blk[:, 0:kw].astype(bf16)

    def prep_wo(nt, z=None):
        nw = 128 if nt < 4 else 64
        wq32[nt, 0:D, 0:nw] = _tie16(wo_v[:, nt * 128:nt * 128 + nw], z).astype(f32)
        for tau in range(5):
            if tau < 4:
                parts = [wq32[nt, pl.ds(4 * tau + g, 32, stride=DH), :] for g in range(4)]
            else:
                parts = [jnp.zeros((64, 128), f32)] + [
                    wq32[nt, pl.ds(16 + g, 32, stride=DH), :] for g in range(2)]
            blk = jnp.concatenate(parts, axis=0)
            wop[tau, nt * 128:nt * 128 + nw, :] = blk.T[0:nw, :].astype(bf16)

    st = {"lo": None}

    def att_a(i, g):
        r = HALO + g * RB
        kv = kvs[i]
        acc = [None] * W
        for t in range(5):
            q = _tie(kv[t, r:r + RB, :], st["lo"])
            for w in range(W):
                p = q * kv[5 + t, r - 2 * w:r - 2 * w + RB, :]
                acc[w] = p if acc[w] is None else acc[w] + p
        return [a + pltpu.roll(a, 64, axis=1) for a in acc]

    def att_b(i, g, acc):
        out = []
        s0 = g * RB if i == 0 else S
        for w in range(W):
            a = acc[w] + pltpu.roll(acc[w], 32, axis=1)
            if s0 < 2 * w:
                row = jax.lax.broadcasted_iota(jnp.int32, (RB, 128), 0)
                a = jnp.where(row >= 2 * w - s0, a, -1e9 / SCALE)
            out.append(a)
        return out

    def att_c(i, g, acc):
        lr = g * RB
        r = HALO + lr
        kv = kvs[i]
        m = acc[0]
        for w in range(1, W):
            m = jnp.maximum(m, acc[w])
        e = [jnp.exp2((a - m) * (SCALE * LOG2E)) for a in acc]
        ssum = e[0]
        for w in range(1, W):
            ssum = ssum + e[w]
        inv = pl.reciprocal(ssum, approx=True)
        inv = inv * (2.0 - ssum * inv)
        for t in range(5):
            o = None
            for w in range(W):
                p = e[w] * kv[(10 + t) if t < 4 else 4, r - 2 * w:r - 2 * w + RB, :]
                o = p if o is None else o + p
            o = o * inv
            if t == 4:
                o = jnp.where(lane >= 64, o, 0.0)
            o_vs[i][t, lr:lr + RB, :] = o.astype(bf16)

    def attn_gen(i):
        sa, sb = {}, {}
        if i > 0:
            kvs[i][4:14, 0:HALO, :] = kvs[i - 1][4:14, SB:SB + HALO, :]
        for step in range(NG + 2):
            if step < NG:
                sa[step] = att_a(i, step)
            if 0 <= step - 1 < NG:
                sb[step - 1] = att_b(i, step - 1, sa.pop(step - 1))
            if 0 <= step - 2 < NG:
                att_c(i, step - 2, sb.pop(step - 2))
            yield

    NS = NG + 2

    def run(gen, n):
        for _ in range(n):
            next(gen, None)

    def wo_ln2(i):
        yT = jax.lax.dot_general(jnp.concatenate([wop[t] for t in range(5)], axis=1),
                                 jnp.concatenate([o_vs[i][t] for t in range(5)], axis=1), NT,
                                 preferred_element_type=f32)
        for t in range(NTB):
            xl = xload(i, t)

            def load1(a, t=t, xl=xl):
                x1 = xl(a) + mod_v[2, a:a + CH, :] * yT[a:a + CH, t * 128:(t + 1) * 128]
                x1_vs[i][t, a:a + CH, :] = x1
                return x1

            def load2(a, t=t):
                return x1_vs[i][t, a:a + CH, :]

            mean, rstd = _ln_stats(load1)
            _ln_apply(load2, mean, rstd, mod_v.at[4], mod_v.at[3], hn_vs[i], t * 128, True)

    def out_copy(i, t, r0=0, r1=D):
        g = i * NTB + t
        return pltpu.make_async_copy(out_v.at[g, pl.ds(r0, r1 - r0), :],
                                     out_hbm.at[pl.ds(r0, r1 - r0), pl.ds(g * 128, 128)], osem)

    def epilogue(i, acc, r0, r1):
        for t in range(NTB):
            for a in range(r0, r1, CH):
                x2 = x1_vs[i][t, a:a + CH, :] + \
                    mod_v[5, a:a + CH, :] * acc[a - r0:a - r0 + CH, t * 128:(t + 1) * 128]
                out_v[i * NTB + t, a:a + CH, :] = x2.astype(bf16)

    def ffn(i):
        last = i == NB - 1
        gen = None if last else attn_gen(i + 1)
        hn = _cat5(hn_vs[i], 0, SB)
        acc = None
        nf = F // FC
        for f in range(nf):
            hp = jnp.dot(hn, w1_v[:, f * FC:(f + 1) * FC], preferred_element_type=f32)
            hh = jnp.maximum(hp, 0.0).astype(bf16)
            if last and f == nf - 1:
                for r0, r1 in RGS:
                    p = jax.lax.dot_general(w2t_v[r0:r1, f * FC:(f + 1) * FC], hh, NT,
                                            preferred_element_type=f32)
                    epilogue(i, acc[r0:r1] + p, r0, r1)
                    for t in range(NTB):
                        out_copy(i, t, r0, r1).start()
                return
            p = jax.lax.dot_general(w2t_v[:, f * FC:(f + 1) * FC], hh, NT,
                                    preferred_element_type=f32)
            acc = p if acc is None else acc + p
            if gen is not None and f < nf - 2:
                zz = [zof(hp[q * SB // 4:q * SB // 4 + 8]) for q in range(4)]
                zz += [zof(p[q * D // 4:q * D // 4 + 8]) for q in range(4)]
                for z in zz:
                    st["lo"] = z
                    run(gen, 1)
            if gen is not None and f == nf - 2:
                st["lo"] = None
                run(gen, NS)
                wo_ln2(i + 1)
        epilogue(i, acc, 0, D)
        for t in range(NTB):
            out_copy(i, t).start()

    lnst = {}
    gen0 = attn_gen(0)

    def dot(i, part, work, rows=None, defer=False):
        n0, n1, tiles = ((0, 512, (0, 1, 2, 3)), (512, 1024, (5, 6, 7, 8)),
                         (1024, 1536, (10, 11, 12, 13)), (1536, 1728, (4, 9)))[part]
        r0, r1 = rows if rows is not None else (0, n1 - n0)
        if r1 - r0 > RS and (r1 - r0) % RS == 0:
            k = (r1 - r0) // RS
            per = max(len(work) // k, 1)
            for j in range(k):
                fin = dot(i, part, work[j * per:(j + 1) * per], rows=(r0 + j * RS, r0 + (j + 1) * RS),
                          defer=(defer and j == k - 1))
            return fin
        hT = jnp.concatenate([h_vs[i][t] for t in range(NTB)], axis=1)
        kv = kvs[i]
        y = jnp.dot(_cat5(wqp, n0 + r0, n0 + r1), hT, preferred_element_type=f32)

        def finish():
            for g0 in range(r0, r1, 128):
                gw = min(128, r1 - g0)
                for t in range(NTB):
                    blk = y[g0 - r0:g0 - r0 + gw, t * 128:(t + 1) * 128]
                    if gw < 128:
                        blk = jnp.concatenate([blk, jnp.zeros((128 - gw, 128), f32)], axis=0)
                    kv[tiles[g0 // 128], HALO + t * 128:HALO + (t + 1) * 128, :] = blk.T
            n, k = r1 - r0, max(len(work), 1)
            for q, items in enumerate(work):
                if items:
                    z = zof(y[q * n // k:q * n // k + 8])
                    for it in items:
                        it(z)

        if defer:
            return finish
        finish()
        return None

    def A1(z):
        st["lo"] = z
        run(gen0, 1)

    def Ls(i, t):
        def f(z):
            lnst[(i, t)] = _ln_stats(xload(i, t), z)
        return f

    def La(i, t):
        def f(z):
            _ln_apply(xload(i, t, zmask if z is None else z), *lnst.pop((i, t)),
                      mod_v.at[1], mod_v.at[0], h_vs[i], t * 128, False)
        return f

    def M(j):
        return lambda z: mod_tile(j, z)

    def PW(p, kt):
        return lambda z: prep_w(p, kt, z)

    def PO(nt):
        return lambda z: prep_wo(nt, z)

    c_wm0.wait()
    for j in range(9):
        mod_tile(j)
    c_x[0].wait()
    for t in range(NTB):
        Ls(0, t)(None)
        La(0, t)(None)
    c_wq.wait()
    for kt in range(5):
        prep_w(0, kt)
    fin = dot(0, 0, [], rows=(0, 256), defer=True)
    c_wk.wait()
    fin()
    dot(0, 0, [[PW(1, kt)] for kt in range(5)], rows=(256, 512))
    fin = dot(0, 1, [], rows=(0, 256), defer=True)
    c_wv.wait()
    fin()
    dot(0, 1, [[PW(2, kt)] for kt in range(5)], rows=(256, 512))
    fin = dot(0, 2, [], rows=(0, 256), defer=True)
    c_x[1].wait()
    c_x[2].wait()
    c_x[3].wait()
    fin()
    dot(0, 2, [[Ls(1, 0)], [La(1, 0)], [Ls(1, 1)], [La(1, 1)]], rows=(256, 512))
    dot(0, 3, [[Ls(1, 2)], [La(1, 2)], [Ls(1, 3)], [La(1, 3)]])
    dot(1, 0, [[A1], [Ls(2, 0)], [A1], [La(2, 0)], [A1], [Ls(2, 1)], [A1], [La(2, 1)]])
    dot(1, 1, [[A1], [Ls(2, 2)], [A1], [La(2, 2)], [A1], [Ls(2, 3)], [A1], [La(2, 3)]])
    dot(1, 2, [[A1], [Ls(3, 0)], [A1], [La(3, 0)], [A1], [Ls(3, 1)], [A1], [La(3, 1)]])
    fin = dot(1, 3, [[A1], [Ls(3, 2)], [A1], [La(3, 2)]], defer=True)
    c_wo.wait()
    c_wm1.wait()
    fin()
    dot(2, 0, [[A1], [Ls(3, 3)], [A1], [La(3, 3)], [A1], [PO(0)], [A1], [PO(1)]])
    dot(2, 1, [[A1], [PO(2)], [A1], [PO(3)], [A1], [PO(4)], [A1], [M(9)]])
    dot(2, 2, [[A1], [M(10)], [A1], [M(11)], [A1], [M(12)], [A1], [M(13)]])
    dot(2, 3, [[A1], [M(14)], [A1], [M(15)]])
    dot(3, 0, [[A1], [M(16)], [A1], [M(17)], [A1], [M(18)], [A1], [M(19)]])
    dot(3, 1, [[A1], [M(20)], [A1], [M(21)], [], [M(22)], [], []])
    st["lo"] = None
    run(gen0, NS)
    wo_ln2(0)
    dot(3, 2, [[], [], [], [M(23)], [], [M(24)], [], []])
    fin = dot(3, 3, [[M(25)], [M(26)]], defer=True)
    c_w1.wait()
    c_w2.wait()
    fin()

    for i in range(NB):
        ffn(i)
    for i in range(NB - 1):
        for t in range(NTB):
            out_copy(i, t).wait()
    for r0, r1 in RGS:
        for t in range(NTB):
            out_copy(NB - 1, t, r0, r1).wait()


@jax.jit
def pallas_adaLN_cond__sliding_local_dilated__dense_activation_relu__prompt_kernel(
    A_x: jax.Array,
    A_wqkv: jax.Array,
    A_wo: jax.Array,
    B_x: jax.Array,
    B_w1: jax.Array,
    B_w2: jax.Array,
    c: jax.Array,
    w_mod: jax.Array,
):
    del B_x
    anyspec = pl.BlockSpec(memory_space=pl.ANY)
    outT = pl.pallas_call(
        _kernel,
        in_specs=[anyspec] * 7,
        out_specs=anyspec,
        out_shape=jax.ShapeDtypeStruct((D, S), bf16),
        scratch_shapes=[
            pltpu.VMEM((NB, D, SB), bf16),
            pltpu.VMEM((D, 3 * D), bf16),
            pltpu.VMEM((D, D), bf16),
            pltpu.VMEM((D, F), bf16),
            pltpu.VMEM((D, F), bf16),
            pltpu.VMEM((D, 6 * D), bf16),
            pltpu.VMEM((S // 128, D, 128), bf16),
            pltpu.VMEM((5, 3 * D, 128), f32),
            pltpu.VMEM((5, 3 * D, 128), bf16),
            pltpu.VMEM((5, D, 128), bf16),
            pltpu.VMEM((6, D, 128), f32),
            pltpu.VMEM((D, 128), f32),
            pltpu.VMEM((1, D), bf16),
            pltpu.SemaphoreType.DMA((9,)),
            pltpu.SemaphoreType.DMA(()),
        ] + [pltpu.VMEM((NTB, D, 128), bf16)] * NB
          + [pltpu.VMEM((14, HALO + SB, 128), f32)] * NB
          + [pltpu.VMEM((5, SB, 128), bf16)] * NB
          + [pltpu.VMEM((NTB, D, 128), f32)] * NB
          + [pltpu.VMEM((5, SB, 128), bf16)] * NB,
        compiler_params=pltpu.CompilerParams(vmem_limit_bytes=100 * 2 ** 20),
        name="adaln_block",
    )(c, A_x.reshape(S, D).T, A_wqkv, A_wo, B_w1, B_w2.T, w_mod)
    return outT.T.reshape(1, S, D)
```

```python
import jax
import jax.numpy as jnp
import jax.experimental.pallas as pl
import jax.experimental.pallas.tpu as pltpu

f32 = jnp.float32
bf16 = jnp.bfloat16
u32 = jnp.uint32

S, D, DH, W, F = 2048, 576, 18, 8, 4608
EPS = 1e-5
SCALE = DH ** -0.5
LOG2E = 1.4426950408889634
NT = (((1,), (1,)), ((), ()))

SB = 512
NB = S // SB
NTB = SB // 128
HALO = 16
RB = 16
NG = SB // RB
FC = 512
CH = 64
RS = 256


def _tie(a, z):
    if z is None:
        return a
    n = a.shape[0] // 8
    a3 = pltpu.bitcast(a, u32).reshape(n, 8, 128) | z[None]
    return pltpu.bitcast(a3.reshape(n * 8, 128), f32)


def _tie16(a, z):
    if z is None:
        return a
    zz = jnp.concatenate([z[:, 0:a.shape[1]]] * (a.shape[0] // 16), axis=0)
    return pltpu.bitcast(pltpu.bitcast(a, u32) | zz, bf16)


def _bc8(row):
    return jnp.broadcast_to(row, (8, 128))


def _rep(a8, n):
    return jnp.concatenate([a8] * (n // 8), axis=0)


def _fold8(a):
    parts = [a[r:r + 8] for r in range(0, a.shape[0], 8)]
    while len(parts) > 1:
        parts = [parts[i] + parts[i + 1] for i in range(0, len(parts), 2)]
    return parts[0]


def _ln_stats(load, z=None):
    x0 = s1 = s2 = None
    for a in range(0, D, CH):
        x = load(a)
        if x0 is None:
            x0 = _tie(_bc8(x[0:1, :]), z)
        d = x - _rep(x0, CH)
        s1 = d if s1 is None else s1 + d
        s2 = d * d if s2 is None else s2 + d * d
    m = jnp.sum(_fold8(s1), axis=0, keepdims=True) * (1.0 / D)
    e2 = jnp.sum(_fold8(s2), axis=0, keepdims=True) * (1.0 / D)
    var = jnp.maximum(e2 - m * m, 0.0)
    return x0 + _bc8(m), _bc8(jax.lax.rsqrt(var + EPS))


def _ln_apply(load, mean, rstd, scale_ref, shift_ref, dst_ref, row0, transpose):
    for c0 in range(0, D, 128):
        cw = min(128, D - c0)
        outs = []
        for a in range(c0, c0 + cw, CH):
            xn = (load(a) - _rep(mean, CH)) * _rep(rstd, CH)
            outs.append(xn * scale_ref[a:a + CH, :] + shift_ref[a:a + CH, :])
        blk = outs[0] if len(outs) == 1 else jnp.concatenate(outs, axis=0)
        if transpose:
            dst_ref[c0 // 128, row0:row0 + 128, 0:cw] = blk.T.astype(bf16)
        else:
            dst_ref[row0 // 128, c0:c0 + cw, :] = blk.astype(bf16)


def _cat5(ref, r0, r1):
    return jnp.concatenate([ref[kt, r0:r1, :] for kt in range(4)] + [ref[4, r0:r1, 0:64]], axis=1)


def _kernel(c_hbm, x_hbm, wqkv_hbm, wo_hbm, w1_hbm, w2t_hbm, wmod_hbm, out_hbm,
            x_v, wqkv_v, wo_v, w1_v, w2t_v, wmod_v, out_v,
            wq32, wqp, wop, wb1, wa2, mod_v, sct_v, c_v, sems, osem, *perblk):
    h_vs, kvs, o_vs, x1_vs, hn_vs, ha_vs = (perblk[k * NB:(k + 1) * NB] for k in range(6))

    def cp(src, dst, i):
        return pltpu.make_async_copy(src, dst, sems.at[i])

    def cols(src, dst, c0, n, i):
        return cp(src.at[:, pl.ds(c0, n)], dst.at[:, pl.ds(c0, n)], i)

    c_c = cp(c_hbm, c_v, 0)
    c_x = [cp(x_hbm.at[:, pl.ds(i * SB, SB)], x_v.at[i], (1, 6, 6, 6)[i]) for i in range(NB)]
    c_wm0 = cols(wmod_hbm, wmod_v, 0, 1152, 2)
    c_wq = cols(wqkv_hbm, wqkv_v, 0, 640, 3)
    c_wk = cols(wqkv_hbm, wqkv_v, 640, 640, 4)
    c_wv = cols(wqkv_hbm, wqkv_v, 1280, 448, 5)
    c_wo = cp(wo_hbm, wo_v, 7)
    c_wm1 = cols(wmod_hbm, wmod_v, 1152, 2304, 7)
    c_w1 = cp(w1_hbm, w1_v, 8)
    c_w2 = cp(w2t_hbm, w2t_v, 8)
    for cc in (c_c, c_wm0, c_x[0], c_wq, c_wk, c_wv, c_x[1], c_x[2], c_x[3], c_wo, c_wm1, c_w1, c_w2):
        cc.start()

    lane = jax.lax.broadcasted_iota(jnp.int32, (RB, 128), 1)
    kvs[0][4:14, 0:HALO, :] = jnp.zeros((10, HALO, 128), f32)

    c_c.wait()
    cf = c_v[...].astype(f32)
    sc = cf * jax.nn.sigmoid(cf)
    c8 = _bc8(cf[:, 0:128])
    zmask = jnp.where((c8 > 1.0) & (c8 < -1.0), jnp.uint32(0xFFFFFFFF), jnp.uint32(0))
    for t in range(5):
        kw = 128 if t < 4 else 64
        row = sc[:, t * 128:t * 128 + kw]
        if kw < 128:
            row = jnp.concatenate([row, jnp.zeros((1, 64), f32)], axis=1)
        sct_v[t * 128:t * 128 + kw, :] = jnp.broadcast_to(row, (128, 128)).T[0:kw, :]

    def zof(val):
        return pltpu.bitcast(val[0:8, 0:128], u32) & zmask

    def mod_tile(j, z=None):
        acc = None
        for a in range(0, D, CH):
            p = wmod_v[a:a + CH, j * 128:(j + 1) * 128].astype(f32) * sct_v[a:a + CH, :]
            acc = _tie(p, z) if acc is None else acc + p
        r = jnp.sum(acc, axis=0, keepdims=True)
        rt = jnp.broadcast_to(r, (128, 128)).T
        g0 = j * 128
        for a in range(g0, g0 + 128, 64):
            jj = a // D
            val = rt[a - g0:a - g0 + 64, :]
            if jj in (1, 4):
                val = val + 1.0
            mod_v[jj, a - jj * D:a - jj * D + 64, :] = val

    def xload(i, t, zb=None):
        def load(a):
            w = x_v[i, a:a + CH, t * 128:(t + 1) * 128]
            if zb is not None:
                w = pltpu.bitcast(pltpu.bitcast(w, u32) | _rep(zb, CH // 2), bf16)
            return w.astype(f32)
        return load

    def prep_w(p, kt, z=None):
        kw = 128 if kt < 4 else 64
        for j in range(*((0, 5), (5, 10), (10, 14))[p]):
            nw = 128 if j < 13 else 64
            t = _tie16(wqkv_v[kt * 128:kt * 128 + kw, j * 128:j * 128 + nw], z).astype(f32).T
            wq32[kt, j * 128:j * 128 + nw, 0:kw] = t
        for d in range(DH):
            if d < 16:
                row0 = p * 512 + d * 32
            elif p == 0:
                row0 = 1536 + (d - 16) * 32
            elif p == 2:
                row0 = 1600 + (d - 16) * 32
            else:
                row0 = 1664 + (d - 16) * 32
            blk = wq32[kt, pl.ds(p * D + d, 32, stride=DH), :]
            wqp[kt, row0:row0 + 32, 0:kw] = blk[:, 0:kw].astype(bf16)

    def prep_wo(nt, z=None):
        nw = 128 if nt < 4 else 64
        wq32[nt, 0:D, 0:nw] = _tie16(wo_v[:, nt * 128:nt * 128 + nw], z).astype(f32)
        for tau in range(5):
            if tau < 4:
                parts = [wq32[nt, pl.ds(4 * tau + g, 32, stride=DH), :] for g in range(4)]
            else:
                parts = [jnp.zeros((64, 128), f32)] + [
                    wq32[nt, pl.ds(16 + g, 32, stride=DH), :] for g in range(2)]
            blk = jnp.concatenate(parts, axis=0)
            wop[tau, nt * 128:nt * 128 + nw, :] = blk[:, 0:nw].T.astype(bf16)

    st = {"lo": None}

    def att_a(i, g):
        r = HALO + g * RB
        kv = kvs[i]
        acc = [None] * W
        for t in range(5):
            q = _tie(kv[t, r:r + RB, :], st["lo"])
            for w in range(W):
                p = q * kv[5 + t, r - 2 * w:r - 2 * w + RB, :]
                acc[w] = p if acc[w] is None else acc[w] + p
        return [a + pltpu.roll(a, 64, axis=1) for a in acc]

    def att_b(i, g, acc):
        out = []
        s0 = g * RB if i == 0 else S
        for w in range(W):
            a = acc[w] + pltpu.roll(acc[w], 32, axis=1)
            if s0 < 2 * w:
                row = jax.lax.broadcasted_iota(jnp.int32, (RB, 128), 0)
                a = jnp.where(row >= 2 * w - s0, a, -1e9 / SCALE)
            out.append(a)
        return out

    def att_c(i, g, acc):
        lr = g * RB
        r = HALO + lr
        kv = kvs[i]
        m = acc[0]
        for w in range(1, W):
            m = jnp.maximum(m, acc[w])
        e = [jnp.exp2((a - m) * (SCALE * LOG2E)) for a in acc]
        ssum = e[0]
        for w in range(1, W):
            ssum = ssum + e[w]
        inv = pl.reciprocal(ssum, approx=True)
        inv = inv * (2.0 - ssum * inv)
        for t in range(5):
            o = None
            for w in range(W):
                p = e[w] * kv[(10 + t) if t < 4 else 4, r - 2 * w:r - 2 * w + RB, :]
                o = p if o is None else o + p
            o = o * inv
            if t == 4:
                o = jnp.where(lane >= 64, o, 0.0)
            o_vs[i][t, lr:lr + RB, :] = o.astype(bf16)

    def attn_gen(i):
        sa, sb = {}, {}
        if i > 0:
            kvs[i][4:14, 0:HALO, :] = kvs[i - 1][4:14, SB:SB + HALO, :]
        for step in range(NG + 2):
            if step < NG:
                sa[step] = att_a(i, step)
            if 0 <= step - 1 < NG:
                sb[step - 1] = att_b(i, step - 1, sa.pop(step - 1))
            if 0 <= step - 2 < NG:
                att_c(i, step - 2, sb.pop(step - 2))
            yield

    NS = NG + 2

    def run(gen, n):
        for _ in range(n):
            next(gen, None)

    def wo_ln2(i):
        yT = jax.lax.dot_general(jnp.concatenate([wop[t] for t in range(5)], axis=1),
                                 jnp.concatenate([o_vs[i][t] for t in range(5)], axis=1), NT,
                                 preferred_element_type=f32)
        for t in range(NTB):
            xl = xload(i, t)

            def load1(a, t=t, xl=xl):
                x1 = xl(a) + mod_v[2, a:a + CH, :] * yT[a:a + CH, t * 128:(t + 1) * 128]
                x1_vs[i][t, a:a + CH, :] = x1
                return x1

            def load2(a, t=t):
                return x1_vs[i][t, a:a + CH, :]

            mean, rstd = _ln_stats(load1)
            _ln_apply(load2, mean, rstd, mod_v.at[4], mod_v.at[3], hn_vs[i], t * 128, True)

    def out_copy(i, t, r0=0, r1=D):
        g = i * NTB + t
        return pltpu.make_async_copy(out_v.at[g, pl.ds(r0, r1 - r0), :],
                                     out_hbm.at[pl.ds(r0, r1 - r0), pl.ds(g * 128, 128)], osem)

    def epilogue(i, acc, r0, r1):
        for t in range(NTB):
            for a in range(r0, r1, 32):
                x2 = x1_vs[i][t, a:a + 32, :] + \
                    mod_v[5, a:a + 32, :] * acc[a - r0:a - r0 + 32, t * 128:(t + 1) * 128]
                out_v[i * NTB + t, a:a + 32, :] = x2.astype(bf16)

    LSUM = (((0, 0), (1, 1), 1), ((1, 0), (1, 1), 1), (0, 0), (1, 1),
            ((0, 0), (0, 1), 1), ((1, 0), (0, 0), -1), ((0, 1), (1, 1), -1))
    RSUM = (((0, 0), (1, 1), 1), (0, 0), ((0, 1), (1, 1), -1), ((1, 0), (0, 0), -1),
            (1, 1), ((0, 0), (0, 1), 1), ((1, 0), (1, 1), 1))
    HM = D // 2

    def comb(x, y, sg):
        return x + y if sg > 0 else x - y

    def sum_blocks(blk, spec, dst, rows, z=None):
        (ra, ca), (rb, cb), sg = spec
        for j in range(2):
            for a in range(0, rows, 32):
                x = _tie16(blk(ra, ca, a, j), z).astype(f32)
                dst[j, a:a + 32, :] = comb(x, blk(rb, cb, a, j).astype(f32), sg).astype(bf16)

    def prep_w1(f, k, z=None):
        blk = lambda r, c, a, j: w1_v[r * 256 + a:r * 256 + a + 32,
                                      f * FC + c * 256 + j * 128:f * FC + c * 256 + (j + 1) * 128]
        sum_blocks(blk, RSUM[k], wb1.at[f, k], 256, z)

    def prep_w2(f, k, z=None):
        blk = lambda r, c, a, j: w2t_v[r * HM + a:r * HM + a + 32,
                                       f * FC + c * 256 + j * 128:f * FC + c * 256 + (j + 1) * 128]
        sum_blocks(blk, LSUM[k], wa2.at[f, k], HM, z)

    def prep_h(i):
        blk = lambda r, c, a, j: hn_vs[i][2 * c + j, r * 256 + a:r * 256 + a + 32, :]
        for k in range(7):
            if len(LSUM[k]) == 3:
                sum_blocks(blk, LSUM[k], ha_vs[i].at[k], 256)

    def cat2(ref):
        return jnp.concatenate([ref[0], ref[1]], axis=1)

    wprep = [(fn, k) for k in range(7) for fn, spec in ((prep_w1, RSUM), (prep_w2, LSUM)) if len(spec[k]) == 3]

    def ffn(i):
        last = i == NB - 1
        gen = None if last else attn_gen(i + 1)
        nf = F // FC

        def lhs1(k):
            if len(LSUM[k]) == 3:
                return cat2(ha_vs[i].at[k])
            r, c = LSUM[k]
            return jnp.concatenate([hn_vs[i][2 * c + j, r * 256:(r + 1) * 256, :] for j in range(2)], axis=1)

        def rhs1(f, k):
            if len(RSUM[k]) == 3:
                return cat2(wb1.at[f, k])
            r, c = RSUM[k]
            return w1_v[r * 256:(r + 1) * 256, f * FC + c * 256:f * FC + (c + 1) * 256]

        def lhs2(f, k):
            if len(LSUM[k]) == 3:
                return cat2(wa2.at[f, k])
            r, c = LSUM[k]
            return w2t_v[r * HM:(r + 1) * HM, f * FC + c * 256:f * FC + (c + 1) * 256]

        acc = [None] * 7

        def first(f):
            rem = jnp.dot(hn_vs[i][4, :, 0:64], w1_v[512:D, f * FC:(f + 1) * FC], preferred_element_type=f32)
            m = [jnp.dot(lhs1(k), rhs1(f, k), preferred_element_type=f32) for k in range(7)]
            r00 = jnp.maximum(rem[0:256, 0:256] + m[0] + m[3] - m[4] + m[6], 0.0)
            r01 = jnp.maximum(rem[0:256, 256:512] + m[2] + m[4], 0.0)
            r10 = jnp.maximum(rem[256:512, 0:256] + m[1] + m[3], 0.0)
            r11 = jnp.maximum(rem[256:512, 256:512] + m[0] - m[1] + m[2] + m[5], 0.0)
            rt = {(0, 0): r00, (0, 1): r10, (1, 0): r01, (1, 1): r11}
            hb = [(comb(rt[s[0]], rt[s[1]], s[2]) if len(s) == 3 else rt[s]).astype(bf16) for s in RSUM]
            return hb, [m[0], m[2], m[4], m[6]]

        def side(f, toks, base):
            for q, v in enumerate(toks):
                z = zof(v)
                if gen is not None and f < nf - 2:
                    st["lo"] = z
                    run(gen, 1)
                if i == 0:
                    fn, g = (prep_w1, f + 2) if base else (prep_w2, f + 1)
                    ks = [k for k in range(7) if len((RSUM if base else LSUM)[k]) == 3]
                    if g < nf:
                        for k in ks[q * 5 // 4:(q + 1) * 5 // 4]:
                            fn(g, k, z)

        nxt = first(0)
        if i == 0:
            for q, (fn, k) in enumerate(wprep):
                fn(1 if fn is prep_w1 else 0, k, zof(nxt[1][q * 4 // len(wprep)]))
        for f in range(nf):
            hb, _ = nxt
            if f + 1 < nf:
                nxt = first(f + 1)
                side(f, nxt[1], True)
            ps = {}
            for k in (0, 2, 3, 4, 6, 1, 5):
                p = jax.lax.dot_general(lhs2(f, k), hb[k], NT, preferred_element_type=f32)
                acc[k] = p if acc[k] is None else acc[k] + p
                ps[k] = p
                if last and f == nf - 1 and k == 6:
                    top = jnp.concatenate([acc[0] + acc[3] - acc[4] + acc[6], acc[2] + acc[4]], axis=1)
                    epilogue(i, top, 0, HM)
                    for t in range(NTB):
                        out_copy(i, t, 0, HM).start()
            side(f, [ps[0], ps[3], ps[6], ps[5]], False)
            if gen is not None and f == nf - 3:
                st["lo"] = None
                run(gen, NS)
                wo_ln2(i + 1)
                prep_h(i + 1)
        if not last:
            top = jnp.concatenate([acc[0] + acc[3] - acc[4] + acc[6], acc[2] + acc[4]], axis=1)
            epilogue(i, top, 0, HM)
        bot = jnp.concatenate([acc[1] + acc[3], acc[0] - acc[1] + acc[2] + acc[5]], axis=1)
        epilogue(i, bot, HM, D)
        for t in range(NTB):
            (out_copy(i, t, HM, D) if last else out_copy(i, t)).start()

    lnst = {}
    gen0 = attn_gen(0)

    def dot(i, part, work, rows=None, defer=False):
        n0, n1, tiles = ((0, 512, (0, 1, 2, 3)), (512, 1024, (5, 6, 7, 8)),
                         (1024, 1536, (10, 11, 12, 13)), (1536, 1728, (4, 9)))[part]
        r0, r1 = rows if rows is not None else (0, n1 - n0)
        if r1 - r0 > RS and (r1 - r0) % RS == 0:
            k = (r1 - r0) // RS
            per = max(len(work) // k, 1)
            for j in range(k):
                fin = dot(i, part, work[j * per:(j + 1) * per], rows=(r0 + j * RS, r0 + (j + 1) * RS),
                          defer=(defer and j == k - 1))
            return fin
        hT = jnp.concatenate([h_vs[i][t] for t in range(NTB)], axis=1)
        kv = kvs[i]
        y = jnp.dot(_cat5(wqp, n0 + r0, n0 + r1), hT, preferred_element_type=f32)

        def finish():
            for g0 in range(r0, r1, 128):
                gw = min(128, r1 - g0)
                for t in range(NTB):
                    blk = y[g0 - r0:g0 - r0 + gw, t * 128:(t + 1) * 128]
                    if gw < 128:
                        blk = jnp.concatenate([blk, jnp.zeros((128 - gw, 128), f32)], axis=0)
                    kv[tiles[g0 // 128], HALO + t * 128:HALO + (t + 1) * 128, :] = blk.T
            n, k = r1 - r0, max(len(work), 1)
            for q, items in enumerate(work):
                if items:
                    z = zof(y[q * n // k:q * n // k + 8])
                    for it in items:
                        it(z)

        if defer:
            return finish
        finish()
        return None

    def A1(z):
        st["lo"] = z
        run(gen0, 1)

    def Ls(i, t):
        def f(z):
            lnst[(i, t)] = _ln_stats(xload(i, t), z)
        return f

    def La(i, t):
        def f(z):
            _ln_apply(xload(i, t, zmask if z is None else z), *lnst.pop((i, t)),
                      mod_v.at[1], mod_v.at[0], h_vs[i], t * 128, False)
        return f

    def M(j):
        return lambda z: mod_tile(j, z)

    def PW(p, kt):
        return lambda z: prep_w(p, kt, z)

    def PO(nt):
        return lambda z: prep_wo(nt, z)

    c_wm0.wait()
    for j in range(9):
        mod_tile(j)
    c_x[0].wait()
    for t in range(NTB):
        Ls(0, t)(None)
        La(0, t)(None)
    c_wq.wait()
    for kt in range(5):
        prep_w(0, kt)
    fin = dot(0, 0, [], rows=(0, 256), defer=True)
    c_wk.wait()
    fin()
    dot(0, 0, [[PW(1, kt)] for kt in range(5)], rows=(256, 512))
    fin = dot(0, 1, [], rows=(0, 256), defer=True)
    c_wv.wait()
    fin()
    dot(0, 1, [[PW(2, kt)] for kt in range(5)], rows=(256, 512))
    fin = dot(0, 2, [], rows=(0, 256), defer=True)
    c_x[1].wait()
    c_x[2].wait()
    c_x[3].wait()
    fin()
    dot(0, 2, [[Ls(1, 0)], [La(1, 0)], [Ls(1, 1)], [La(1, 1)]], rows=(256, 512))
    dot(0, 3, [[Ls(1, 2)], [La(1, 2)], [Ls(1, 3)], [La(1, 3)]])
    dot(1, 0, [[A1], [Ls(2, 0)], [A1], [La(2, 0)], [A1], [Ls(2, 1)], [A1], [La(2, 1)]])
    dot(1, 1, [[A1], [Ls(2, 2)], [A1], [La(2, 2)], [A1], [Ls(2, 3)], [A1], [La(2, 3)]])
    dot(1, 2, [[A1], [Ls(3, 0)], [A1], [La(3, 0)], [A1], [Ls(3, 1)], [A1], [La(3, 1)]])
    fin = dot(1, 3, [[A1], [Ls(3, 2)], [A1], [La(3, 2)]], defer=True)
    c_wo.wait()
    c_wm1.wait()
    fin()
    dot(2, 0, [[A1], [Ls(3, 3)], [A1], [La(3, 3)], [A1], [PO(0)], [A1], [PO(1)]])
    dot(2, 1, [[A1], [PO(2)], [A1], [PO(3)], [A1], [PO(4)], [A1], [M(9)]])
    dot(2, 2, [[A1], [M(10)], [A1], [M(11)], [A1], [M(12)], [A1], [M(13)]])
    dot(2, 3, [[A1], [M(14)], [A1], [M(15)]])
    dot(3, 0, [[A1], [M(16)], [A1], [M(17)], [A1], [M(18)], [A1], [M(19)]])
    dot(3, 1, [[A1], [M(20)], [A1], [M(21)], [], [M(22)], [], []])
    st["lo"] = None
    run(gen0, NS)
    wo_ln2(0)
    prep_h(0)
    fin = dot(3, 2, [[], [M(23)], [], [M(24)], [M(25)], [M(26)], [], []], defer=True)
    c_w1.wait()
    c_w2.wait()
    fin()
    dot(3, 3, [[lambda z, k=k: prep_w1(0, k, z)] for k in range(7) if len(RSUM[k]) == 3])

    for i in range(NB):
        ffn(i)
    for i in range(NB - 1):
        for t in range(NTB):
            out_copy(i, t).wait()
    for r0, r1 in ((0, HM), (HM, D)):
        for t in range(NTB):
            out_copy(NB - 1, t, r0, r1).wait()


@jax.jit
def pallas_adaLN_cond__sliding_local_dilated__dense_activation_relu__prompt_kernel(
    A_x: jax.Array,
    A_wqkv: jax.Array,
    A_wo: jax.Array,
    B_x: jax.Array,
    B_w1: jax.Array,
    B_w2: jax.Array,
    c: jax.Array,
    w_mod: jax.Array,
):
    del B_x
    anyspec = pl.BlockSpec(memory_space=pl.ANY)
    outT = pl.pallas_call(
        _kernel,
        in_specs=[anyspec] * 7,
        out_specs=anyspec,
        out_shape=jax.ShapeDtypeStruct((D, S), bf16),
        scratch_shapes=[
            pltpu.VMEM((NB, D, SB), bf16),
            pltpu.VMEM((D, 3 * D), bf16),
            pltpu.VMEM((D, D), bf16),
            pltpu.VMEM((D, F), bf16),
            pltpu.VMEM((D, F), bf16),
            pltpu.VMEM((D, 6 * D), bf16),
            pltpu.VMEM((S // 128, D, 128), bf16),
            pltpu.VMEM((5, 3 * D, 128), f32),
            pltpu.VMEM((5, 3 * D, 128), bf16),
            pltpu.VMEM((5, D, 128), bf16),
            pltpu.VMEM((F // FC, 7, 2, 256, 128), bf16),
            pltpu.VMEM((F // FC, 7, 2, D // 2, 128), bf16),
            pltpu.VMEM((6, D, 128), f32),
            pltpu.VMEM((D, 128), f32),
            pltpu.VMEM((1, D), bf16),
            pltpu.SemaphoreType.DMA((9,)),
            pltpu.SemaphoreType.DMA(()),
        ] + [pltpu.VMEM((NTB, D, 128), bf16)] * NB
          + [pltpu.VMEM((14, HALO + SB, 128), f32)] * NB
          + [pltpu.VMEM((5, SB, 128), bf16)] * NB
          + [pltpu.VMEM((NTB, D, 128), f32)] * NB
          + [pltpu.VMEM((5, SB, 128), bf16)] * NB
          + [pltpu.VMEM((7, 2, 256, 128), bf16)] * NB,
        compiler_params=pltpu.CompilerParams(vmem_limit_bytes=100 * 2 ** 20),
        name="adaln_block",
    )(c, A_x.reshape(S, D).T, A_wqkv, A_wo, B_w1, B_w2.T, w_mod)
    return outT.T.reshape(1, S, D)
```
